```python
import os as _os
_os.environ.setdefault("JAX_PLATFORMS", "cpu")
import jax
import jax.numpy as jnp

def _softmax(x, axis=-1):
    return jax.nn.softmax(x, axis=axis)
def _gelu(x):
    return jax.nn.gelu(x, approximate=True)
def _silu(x):
    return jax.nn.silu(x)
def _sigmoid(x):
    return jax.nn.sigmoid(x)
def _layernorm(x, axis=-1, eps=1e-5):
    m = jnp.mean(x, axis=axis, keepdims=True)
    v = jnp.var(x, axis=axis, keepdims=True)
    return (x - m) / jnp.sqrt(v + eps)
def _scatter_add(tgt, idx, src, axis=0):
    return tgt.at[idx].add(src)
def _segment_sum(src, seg, n):
    return jax.ops.segment_sum(src, seg, n)
class _Rng:
    def __init__(self, key):
        self._k = key
    def _next(self):
        self._k, sub = jax.random.split(self._k)
        return sub
    def normal(self, shape):
        return jax.random.normal(self._next(), shape, dtype=jnp.bfloat16)
    def randint(self, lo, hi, shape):
        return jax.random.randint(self._next(), shape, lo, hi, dtype=jnp.int32)
    def uniform(self, shape, lo=0.0, hi=1.0):
        return jax.random.uniform(self._next(), shape, jnp.bfloat16, lo, hi)
    def permutation(self, n):
        return jax.random.permutation(self._next(), n)


kernel_name = 'concat_heads__mha_block_cached__gqa_block_cached__decode'

def setup_inputs():
    _rng = _Rng(jax.random.key(int.from_bytes(__import__("os").urandom(4), "little")))
    _w = (lambda a: (lambda t: t.astype(jnp.bfloat16) if jnp.issubdtype(t.dtype, jnp.floating) else t)(jnp.asarray(a)))
    def _A_setup():
        B, Sq, D = 1, 1, 512
        H, Sk, Dh = 32, 4096, 128
        return {
            "x": _w((lambda *s: _rng.normal(s) * 0.8)(B, Sq, D)),
            "k_cache": _w((lambda *s: _rng.normal(s) * 0.8)(B, H, Sk, Dh)),
            "v_cache": _w((lambda *s: _rng.normal(s) * 0.05)(B, H, Sk, Dh)),
            "wq": _w((lambda *s: _rng.normal(s) * 0.8)(D, H * Dh) * (D ** -0.5)),
            "wo": _w((lambda *s: _rng.normal(s) * 0.05)(H * Dh, D) * ((H * Dh) ** -0.5)),
        }
    _A_in = _A_setup()

    def _B_setup():
        B, Sq, D = 1, 1, 512
        Hq, Hkv, Sk, Dh = 32, 32, 4096, 128
        assert Hq % Hkv == 0, (Hq, Hkv)
        return {
            "x": _w((lambda *s: _rng.normal(s) * 0.8)(B, Sq, D)),
            "k_cache": _w((lambda *s: _rng.normal(s) * 0.8)(B, Hkv, Sk, Dh)),
            "v_cache": _w((lambda *s: _rng.normal(s) * 0.05)(B, Hkv, Sk, Dh)),
            "wq": _w((lambda *s: _rng.normal(s) * 0.8)(D, Hq * Dh) * (D ** -0.5)),
            "wo": _w((lambda *s: _rng.normal(s) * 0.05)(Hq * Dh, D) * ((Hq * Dh) ** -0.5)),
        }
    _B_in = _B_setup()

    return {
        "A_x": _A_in["x"],
        "A_k_cache": _A_in["k_cache"],
        "A_v_cache": _A_in["v_cache"],
        "A_wq": _A_in["wq"],
        "A_wo": _A_in["wo"],
        "B_x": _B_in["x"],
        "B_k_cache": _B_in["k_cache"],
        "B_v_cache": _B_in["v_cache"],
        "B_wq": _B_in["wq"],
        "B_wo": _B_in["wo"],
    }

def reference(A_x, A_k_cache, A_v_cache, A_wq, A_wo, B_x, B_k_cache, B_v_cache, B_wq, B_wo):
    def _A_ref(x, k_cache, v_cache, wq, wo):
        B, Sq, D = x.shape
        H, Dh = 32, 128
        q = (lambda x, *d: x.transpose(*d))((x @ wq).reshape(B, Sq, H, Dh), 0, 2, 1, 3)
        scores = jnp.einsum("bhqd,bhkd->bhqk", q, k_cache) * (Dh ** -0.5)
        p = _softmax(scores, axis=-1)
        o = jnp.einsum("bhqk,bhkd->bhqd", p, v_cache)
        return (lambda x, *d: x.transpose(*d))(o, 0, 2, 1, 3).reshape(B, Sq, H * Dh) @ wo

    def _B_ref(x, k_cache, v_cache, wq, wo):
        B, Sq, D = x.shape
        Hq, Dh = 32, 128
        Hkv = k_cache.shape[1]
        rep = Hq // Hkv
        q = (lambda x, *d: x.transpose(*d))((x @ wq).reshape(B, Sq, Hq, Dh), 0, 2, 1, 3)
        k = jnp.repeat(k_cache, rep, axis=1)
        v = jnp.repeat(v_cache, rep, axis=1)
        scores = jnp.einsum("bhqd,bhkd->bhqk", q, k) * (Dh ** -0.5)
        p = _softmax(scores, axis=-1)
        o = jnp.einsum("bhqk,bhkd->bhqd", p, v)
        return (lambda x, *d: x.transpose(*d))(o, 0, 2, 1, 3).reshape(B, Sq, Hq * Dh) @ wo

    a = _A_ref(A_x, A_k_cache, A_v_cache, A_wq, A_wo)
    b = _B_ref(B_x, B_k_cache, B_v_cache, B_wq, B_wo)
    return jnp.concatenate([a, b], axis=-1)
```

```python
import functools
import jax
import jax.numpy as jnp
from jax import lax
import jax.experimental.pallas as pl
import jax.experimental.pallas.tpu as pltpu

H, SK, DH, D = 32, 4096, 128, 512
NS = 8
R1, R0 = 384, 128
P0_BASE = NS * R1
WQ_ROWS = 8
WQ_N = D // WQ_ROWS
WQ_D = 8
WO0 = 32
E_P0_HEADS = 8
E_N1 = H - E_P0_HEADS
BULK, PACED = 1, 0
SCALE = DH ** -0.5
f32, bf16 = jnp.float32, jnp.bfloat16


def _kernel(ax, ak, av, awq, awo, bx, bk, bv, bwq, bwo, o_ref,
            xbuf, wqbuf, wobuf, kvbuf, qbuf, sbuf, obuf, lbuf, onbuf):
    kv_src = (ak, av, bk, bv)
    wq_src = (awq, bwq)

    def inner(xsem, wqsem, woasem, sem1, sem0, esem1, esem0):
        def c1(a, h, s):
            rows = pl.ds(pl.multiple_of(s * R1, R1), R1)
            return pltpu.make_async_copy(kv_src[a].at[0, h, rows], kvbuf.at[a, rows], sem1.at[a, s])

        def c0(a, h, s):
            rows = pl.ds(pl.multiple_of(P0_BASE + s * R0, R0), R0)
            return pltpu.make_async_copy(kv_src[a].at[0, h, rows], kvbuf.at[a, rows], sem0.at[a])

        def c0_wait_all(a):
            reg = kvbuf.at[a, pl.ds(P0_BASE, NS * R0)]
            pltpu.make_async_copy(reg, reg, sem0.at[a]).wait()

        def cwq(b, i):
            rows = pl.ds(pl.multiple_of(i * WQ_ROWS, WQ_ROWS), WQ_ROWS)
            return pltpu.make_async_copy(wq_src[b].at[rows], wqbuf.at[b, rows], wqsem.at[b, i % WQ_D])

        def cwoa(i):
            rows = pl.ds(pl.multiple_of(i * WO0, WO0), WO0)
            return pltpu.make_async_copy(awo.at[rows], wobuf.at[0, rows], woasem)

        def ce1(j):
            rows = pl.ds(pl.multiple_of((E_P0_HEADS + j) * DH, DH), DH)
            return pltpu.make_async_copy(bwo.at[rows], wobuf.at[1, rows], esem1.at[j])

        def ce0(i):
            rows = pl.ds(pl.multiple_of(i * WO0, WO0), WO0)
            return pltpu.make_async_copy(bwo.at[rows], wobuf.at[1, rows], esem0.at[i // 4])

        def ce0_wait_head(g):
            reg = wobuf.at[1, pl.ds(g * DH, DH)]
            pltpu.make_async_copy(reg, reg, esem0.at[g]).wait()

        cx = [pltpu.make_async_copy(x, xbuf.at[i], xsem.at[i]) for i, x in enumerate((ax, bx))]

        for i in range(WQ_D):
            for b in range(2):
                cwq(b, i).start(priority=BULK)
        for c in cx:
            c.start(priority=PACED)

        def wstep(i, c, tail):
            for b in range(2):
                cwq(b, i).wait()
                cwoa(2 * i + b).start(priority=PACED)
                if tail:
                    s = i - (WQ_N - WQ_D)
                    c1(b, 0, s).start(priority=BULK)
                    c0(b, 0, s).start(priority=BULK)
                else:
                    cwq(b, i + WQ_D).start(priority=BULK)
            return c

        lax.fori_loop(0, WQ_N - WQ_D, functools.partial(wstep, tail=False), 0)
        lax.fori_loop(WQ_N - WQ_D, WQ_N, functools.partial(wstep, tail=True), 0)

        for b in range(2):
            cx[b].wait()
            x8 = jnp.broadcast_to(xbuf[b, 0], (8, D))
            q = jnp.dot(x8, wqbuf[b], preferred_element_type=f32).astype(bf16)
            for h in range(H):
                qbuf[b, h] = q[:, h * DH:(h + 1) * DH]

        def blk(a, s):
            r1 = kvbuf[a, pl.ds(pl.multiple_of(s * R1, R1), R1), :]
            r0 = kvbuf[a, pl.ds(pl.multiple_of(P0_BASE + s * R0, R0), R0), :]
            return jnp.concatenate([r1, r0], axis=0)

        def fold(x, op):
            r = x[:, 0:DH]
            for t in range(1, (R1 + R0) // DH):
                r = op(r, x[:, t * DH:(t + 1) * DH])
            return r

        def head(h, last):
            def issue(a, s):
                if a < 2:
                    c0(a + 2, h, s).start(priority=PACED)
                    c1(a + 2, h, s).start(priority=BULK)
                elif not last:
                    c0(a - 2, h + 1, s).start(priority=PACED)
                    c1(a - 2, h + 1, s).start(priority=BULK)
                else:
                    j = (a - 2) * NS + s
                    ce0(j).start(priority=PACED)
                    ce1(j).start(priority=BULK)

            for b in range(2):
                ka, va = 2 * b, 2 * b + 1
                q = qbuf[b, h]
                c0_wait_all(ka)

                def kstep(s, m_run):
                    c1(ka, h, s).wait()
                    issue(ka, s)
                    sc = lax.dot_general(q, blk(ka, s), (((1,), (1,)), ((), ())), preferred_element_type=f32)
                    sbuf[s] = sc
                    return jnp.maximum(m_run, fold(sc, jnp.maximum))

                m_run = lax.fori_loop(0, NS, kstep, jnp.full((8, DH), -jnp.inf, f32))
                m = jnp.max(m_run, axis=-1, keepdims=True)
                c0_wait_all(va)

                def vstep(s, carry):
                    acc, l_run = carry
                    c1(va, h, s).wait()
                    issue(va, s)
                    p = jnp.exp((sbuf[s] - m) * SCALE)
                    acc = acc + jnp.dot(p.astype(bf16), blk(va, s), preferred_element_type=f32)
                    return acc, l_run + fold(p, jnp.add)

                z = jnp.zeros((8, DH), f32)
                acc, l_run = lax.fori_loop(0, NS, vstep, (z, z))
                obuf[pl.ds(b * H + h, 1), :] = acc[0:1]
                lbuf[pl.ds(b * H + h, 1), :] = l_run[0:1]

        def body(h, c):
            head(h, False)
            return c

        lax.fori_loop(0, H - 1, body, 0)
        head(H - 1, True)

        onbuf[...] = obuf[...] / jnp.sum(lbuf[...], axis=-1, keepdims=True)

        def orow(idx):
            return jnp.broadcast_to(onbuf[idx:idx + 1, :], (8, DH)).astype(bf16)

        pltpu.make_async_copy(wobuf.at[0], wobuf.at[0], woasem).wait()
        oa = jnp.concatenate([orow(h) for h in range(H)], axis=1)
        outa = jnp.dot(oa, wobuf[0], preferred_element_type=f32)
        o_ref[0, :, 0:D] = outa[0:1].astype(o_ref.dtype)

        acc = jnp.zeros((8, D), f32)
        n0 = 4 * E_P0_HEADS
        done0 = 0
        for j in range(E_N1):
            ce1(j).wait()
            if 2 * NS + j < n0:
                ce0(2 * NS + j).start(priority=PACED)
            if j + 2 * NS < E_N1:
                ce1(j + 2 * NS).start(priority=BULK)
            hh = E_P0_HEADS + j
            acc = acc + jnp.dot(orow(H + hh), wobuf[1, hh * DH:(hh + 1) * DH, :], preferred_element_type=f32)
            if done0 < E_P0_HEADS and j >= 4 * done0 + 3 - 2 * NS + 4:
                g = done0
                ce0_wait_head(g)
                acc = acc + jnp.dot(orow(H + g), wobuf[1, g * DH:(g + 1) * DH, :], preferred_element_type=f32)
                done0 += 1
        assert done0 == E_P0_HEADS
        o_ref[0, :, D:2 * D] = acc[0:1].astype(o_ref.dtype)

    dma = pltpu.SemaphoreType.DMA
    pl.run_scoped(inner, dma((2,)), dma((2, WQ_D)), dma(()), dma((4, NS)), dma((4,)), dma((E_N1,)), dma((E_P0_HEADS,)))


@jax.jit
def pallas_concat_heads__mha_block_cached__gqa_block_cached__decode_kernel(
    A_x, A_k_cache, A_v_cache, A_wq, A_wo, B_x, B_k_cache, B_v_cache, B_wq, B_wo):
    return pl.pallas_call(
        _kernel,
        in_specs=[pl.BlockSpec(memory_space=pl.ANY)] * 10,
        out_specs=pl.BlockSpec(memory_space=pltpu.VMEM),
        out_shape=jax.ShapeDtypeStruct((1, 1, 2 * D), bf16),
        scratch_shapes=[
            pltpu.VMEM((2, 1, 1, D), bf16),
            pltpu.VMEM((2, D, H * DH), bf16),
            pltpu.VMEM((2, H * DH, D), bf16),
            pltpu.VMEM((4, SK, DH), bf16),
            pltpu.VMEM((2, H, 8, DH), bf16),
            pltpu.VMEM((NS, 8, R1 + R0), f32),
            pltpu.VMEM((2 * H, DH), f32),
            pltpu.VMEM((2 * H, DH), f32),
            pltpu.VMEM((2 * H, DH), f32),
        ],
        compiler_params=pltpu.CompilerParams(vmem_limit_bytes=64 * 1024 * 1024),
    )(A_x, A_k_cache, A_v_cache, A_wq, A_wo, B_x, B_k_cache, B_v_cache, B_wq, B_wo)
```

```python
import functools

import jax
import jax.numpy as jnp
from jax import lax
import jax.experimental.pallas as pl
import jax.experimental.pallas.tpu as pltpu

H, SK, DH, D = 32, 4096, 128, 512
SCALE = DH ** -0.5
f32, bf16 = jnp.float32, jnp.bfloat16

BULK, PACED = 1, 0
TK = SK // 8
TW = DH * D // (8 * DH)
HS = 16
ST = 9
CUT = (14, 15)
WQ_ROWS = 16
WQ_N = D // WQ_ROWS
RING = 16
KSTEPS = 3
AHEAD = 3 * KSTEPS
NL0, NM = 4, 4
VP = (96, 32)
NL = NL0 + NM + 1
NE = H - NL
EB = 3


def _pattern(n, gap, rest, cut):
    ch = []
    for i in range(n):
        ch += [gap + (1 if i == 0 else 0), rest - (cut if i == n - 1 else 0)]
    return tuple(ch)


CH_MAIN = (_pattern(ST, 11, 37, 16), _pattern(ST, 11, 37, 10))
CH_WARM = _pattern(2, 14, 41, 7)
CH_WARM_KV = _pattern(ST // KSTEPS, 11, 40, 6)
CH_LATE = _pattern(2 * NL0, 14, 37, 6)
assert NE == WQ_N - AHEAD and ST % KSTEPS == 0 and sum(VP) == DH
assert all(0 < c < HS for c in CUT)


def _aligned(i, n):
    return i if isinstance(i, int) else pl.multiple_of(i, n)


def _tick(ref):
    return ref.at[ref.shape[0] - 1]


def _spin(tick, n):
    t = tick[...].astype(f32)
    for _ in range(n):
        t = t * 0.5 + 1.0
    tick[...] = t.astype(bf16)


def _track(paced, bulk, tick, ch):
    for k in range(len(ch)):
        paced(k)
        if k == 1 and bulk is not None:
            bulk()
        _spin(tick, ch[k])


def _wait(region, sem):
    pltpu.make_async_copy(region, region, sem).wait()


def _kernel(ax, ak, av, awq, awo, bx, bk, bv, bwq, bwo, o_ref,
            xbuf, x8, wqa, wqb, woa, wob, wol, kv0, kv1, kv2, kv3, pbuf, obuf, ocol):
    kv_src, kvb = (ak, av, bk, bv), (kv0, kv1, kv2, kv3)
    wq_src, wqs, wos = (awq, bwq), (wqa, wqb), (woa, wob)

    def body(xsem, wqsem, wosem, kvsem, hsem, lsem0, lsem1, vsem):
        def kv_copy(a, src, dst, n, sem):
            return pltpu.make_async_copy(kv_src[a].at[pl.ds(src, n)], kvb[a].at[pl.ds(dst, n)], sem)

        def kv_lead(a, h, sem):
            return kv_copy(a, h * TK, (h % 2) * TK, CUT[a // 2], sem)

        def kv_window(a, h):
            return pl.ds((h % 2) * CUT[a // 2], TK)

        def kv_bulk(a, h):
            t0 = CUT[a // 2] + 2 * HS * ST
            kv_copy(a, h * TK + t0, t0, TK - t0, kvsem.at[a]).start(priority=BULK)
            if isinstance(h, int):
                if h + 1 < H:
                    kv_lead(a, h + 1, kvsem.at[a]).start(priority=BULK)
            else:
                @pl.when(h + 1 < H)
                def _():
                    kv_lead(a, h + 1, kvsem.at[a]).start(priority=BULK)

        def kv_paced(a, h, j):
            t0 = CUT[a // 2] + j * HS
            kv_copy(a, h * TK + t0, t0, HS, kvsem.at[a]).start(priority=PACED)

        def kv_load(a, h):
            return kvb[a][kv_window(a, h)].reshape(SK, DH)

        def wo_load(ref, h, n=1):
            w = ref[pl.ds(h * TW, n * TW)].reshape(n * DH // 8, D // DH, 8, DH)
            return jnp.concatenate([w[:, t].reshape(n * DH, DH) for t in range(D // DH)], axis=1)

        def wq_copy(b, i):
            rows = pl.ds(_aligned(i * WQ_ROWS, WQ_ROWS), WQ_ROWS)
            return pltpu.make_async_copy(wq_src[b].at[rows], wqs[b].at[rows], wqsem.at[i % RING])

        def wo_copy(src, dst, t0, n, sem):
            return pltpu.make_async_copy(src.at[pl.ds(t0, n)], dst.at[pl.ds(t0, n)], sem)

        def wo_paced(src, dst, t0, nstripes, j, half, may_wrap, sem, cut):
            if half == 0:
                wo_copy(src, dst, t0 + 2 * HS * j + cut, 2 * HS - cut, sem).start(priority=PACED)
            else:
                nx = j + 1
                if isinstance(nx, int):
                    nx = nx % nstripes
                elif may_wrap:
                    nx = jnp.where(nx == nstripes, 0, nx)
                wo_copy(src, dst, t0 + 2 * HS * nx, cut, sem).start(priority=PACED)

        def late_copy(r, n, sem):
            return wo_copy(bwo, wol, r * TW // DH, n * TW // DH, sem)

        late_mxu = [late_copy((NL0 + j) * DH, DH, lsem1.at[j]) for j in range(NM)]
        late_vpu = [late_copy((NL - 1) * DH + sum(VP[:i]), VP[i], vsem.at[i]) for i in range(len(VP))]
        x_copy = [pltpu.make_async_copy(x, xbuf.at[i], xsem.at[i]) for i, x in enumerate((ax, bx))]

        def qproj(b, h):
            w = wqs[b][:, pl.ds(_aligned(h * DH, DH), DH)]
            return jnp.dot(x8[b], w, preferred_element_type=f32).astype(bf16)

        for i in range(AHEAD):
            wq_copy(0, i).start(priority=BULK)
        for c in x_copy:
            c.start(priority=PACED)
        for r in kvb + (woa, wob, wol):
            _tick(r)[...] = jnp.zeros((8, DH), bf16)

        def warm(lo, hi, b, paced, bulk, tick, ch):
            def step(i, c):
                wq_copy(b, i).wait()
                _track(functools.partial(paced, i), bulk and functools.partial(bulk, i), tick, ch)
                return c
            lax.fori_loop(lo, hi, step, 0)

        def woa_paced(i, k):
            wo_paced(awo, woa, 0, 2 * H, 2 * i + k // 2, k % 2, k == 3, wosem.at[0], CUT[0])

        def wob_paced(i, k):
            wo_paced(bwo, wob, NL * TW, 2 * NE, 2 * i + k // 2, k % 2, k == 3, wosem.at[1], CUT[1])

        warm(0, WQ_N - AHEAD, 0, woa_paced,
             lambda i: wq_copy(0, i + AHEAD).start(priority=BULK), _tick(woa), CH_WARM)
        for b in range(2):
            x_copy[b].wait()
            x8[b] = jnp.broadcast_to(xbuf[b, 0], (8, D))
        warm(WQ_N - AHEAD, WQ_N, 0, woa_paced,
             lambda i: wq_copy(1, i + AHEAD - WQ_N).start(priority=BULK), _tick(woa), CH_WARM)
        q0 = qproj(0, 0)
        lead0 = [kv_lead(a, 0, hsem.at[a]) for a in range(4)]
        for c in lead0:
            c.start(priority=BULK)
        warm(0, NE, 1, wob_paced,
             lambda i: wq_copy(1, i + AHEAD).start(priority=BULK), _tick(wob), CH_WARM)
        for a in range(3):
            lo = NE + a * KSTEPS
            kv_bulk(a, 0)
            warm(lo, lo + KSTEPS, 1,
                 lambda i, k: kv_paced(a, 0, len(CH_WARM_KV) * (i - lo) + k),
                 None, _tick(kvb[a]), CH_WARM_KV)
        for c in lead0:
            c.wait()
        _wait(woa.at[pl.ds(0, H * TW)], wosem.at[0])
        _wait(wob.at[pl.ds(NL * TW, NE * TW)], wosem.at[1])

        def head(h, carry, last):
            q, outs = carry[0], list(carry[1:])

            def begin(a):
                rows = pl.ds(CUT[a // 2], TK - CUT[a // 2]) if last else kv_window(a, h + 1)
                _wait(kvb[a].at[rows], kvsem.at[a])
                if a == 0 or not last:
                    na, nh = (3, h) if a == 0 else (a - 1, h + 1)
                    _track(functools.partial(kv_paced, na, nh), functools.partial(kv_bulk, na, nh),
                           _tick(kvb[na]), CH_MAIN[a % 2])
                elif a == 1:
                    def late_bulk():
                        for c in late_mxu + late_vpu:
                            c.start(priority=BULK)
                    _track(lambda k: wo_paced(bwo, wol, 0, 2 * NL0, k // 2, k % 2, True, lsem0, CUT[1]),
                           late_bulk, _tick(wol), CH_LATE)

            for b in range(2):
                final = last and b == 1
                begin(2 * b)
                s = lax.dot_general(q, kv_load(2 * b, h), (((1,), (1,)), ((), ())),
                                    preferred_element_type=f32)
                m = jnp.max(s, axis=-1, keepdims=True)
                p = jnp.exp((s - m) * SCALE)
                l = jnp.sum(p, axis=-1, keepdims=True)
                pbuf[...] = p.astype(bf16)

                if final:
                    _wait(wol.at[pl.ds(0, NL0 * TW)], lsem0)
                begin(2 * b + 1)
                if final:
                    lhs = jnp.concatenate([obuf[g] for g in range(NL0)], axis=1)
                    outs[1] = outs[1] + jnp.dot(lhs, wo_load(wol, 0, NL0), preferred_element_type=f32)
                o = jnp.dot(pbuf[...], kv_load(2 * b + 1, h), preferred_element_type=f32) / l
                if final:
                    return o, outs
                q = qproj(1, h) if b == 0 else qproj(0, h + 1)
                if b == 0:
                    hw, ow = h, o
                else:
                    obuf[h] = o.astype(bf16)
                    hw, ow = jnp.maximum(h, NL), jnp.where(h >= NL, o, 0.0)
                w = wo_load(wos[b], hw)
                outs[b] = outs[b] + jnp.dot(ow.astype(bf16), w, preferred_element_type=f32)
            return (q, *outs)

        z = jnp.zeros((8, D), f32)
        carry = lax.fori_loop(0, H - 1, lambda h, c: head(h, c, False), (q0, z, z))
        ocol[...] = jnp.broadcast_to(obuf[NL - 1][0:1].astype(f32), (DH, DH)).T
        o_last, (outa, acc) = head(H - 1, carry, True)

        o_ref[0, :, 0:D] = outa[0:1].astype(o_ref.dtype)
        for c in late_mxu[:EB]:
            c.wait()
        lhs = jnp.concatenate([obuf[g] for g in range(NL0, NL0 + EB)] + [o_last.astype(bf16)], axis=1)
        rhs = jnp.concatenate([wo_load(wol, NL0, EB), wo_load(wob, H - 1)], axis=0)
        acc = acc + jnp.dot(lhs, rhs, preferred_element_type=f32)
        for j in range(EB, NM):
            late_mxu[j].wait()
            g = NL0 + j
            acc = acc + jnp.dot(obuf[g], wo_load(wol, g), preferred_element_type=f32)
        acc = jnp.where(lax.broadcasted_iota(jnp.int32, (8, D), 0) == 0, acc, 0.0)
        for i, c in enumerate(late_vpu):
            c.wait()
            for r in range(sum(VP[:i]), sum(VP[:i + 1]), 8):
                t0 = (NL - 1) * TW + r // 8 * (D // DH)
                oc = ocol[r:r + 8, :]
                acc = acc + jnp.concatenate([wol[t0 + t].astype(f32) * oc for t in range(D // DH)], axis=1)
        o_ref[0, :, D:2 * D] = jnp.sum(acc, axis=0, keepdims=True).astype(o_ref.dtype)

    dma = pltpu.SemaphoreType.DMA
    pl.run_scoped(body, dma((2,)), dma((RING,)), dma((2,)), dma((4,)), dma((4,)), dma(()), dma((NM,)),
                  dma((len(VP),)))


@jax.jit
def pallas_concat_heads__mha_block_cached__gqa_block_cached__decode_kernel(
    A_x: jax.Array,
    A_k_cache: jax.Array,
    A_v_cache: jax.Array,
    A_wq: jax.Array,
    A_wo: jax.Array,
    B_x: jax.Array,
    B_k_cache: jax.Array,
    B_v_cache: jax.Array,
    B_wq: jax.Array,
    B_wo: jax.Array,
):
    for x, k, v, wq, wo in ((A_x, A_k_cache, A_v_cache, A_wq, A_wo),
                            (B_x, B_k_cache, B_v_cache, B_wq, B_wo)):
        assert x.shape == (1, 1, D) and k.shape == v.shape == (1, H, SK, DH)
        assert wq.shape == (D, H * DH) and wo.shape == (H * DH, D)
    kv_t = lambda a: a.reshape(H * TK, 8, DH)
    wo_t = lambda w: w.reshape(H * DH // 8, 8, D // DH, DH).transpose(0, 2, 1, 3).reshape(H * TW, 8, DH)
    kv_buf = pltpu.VMEM((TK + HS, 8, DH), bf16)
    return pl.pallas_call(
        _kernel,
        in_specs=[pl.BlockSpec(memory_space=pl.ANY)] * 10,
        out_specs=pl.BlockSpec(memory_space=pltpu.VMEM),
        out_shape=jax.ShapeDtypeStruct((1, 1, 2 * D), bf16),
        scratch_shapes=[
            pltpu.VMEM((2, 1, 1, D), bf16),
            pltpu.VMEM((2, 8, D), bf16),
            pltpu.VMEM((D, H * DH), bf16),
            pltpu.VMEM((D, H * DH), bf16),
            pltpu.VMEM((H * TW + 1, 8, DH), bf16),
            pltpu.VMEM((H * TW + 1, 8, DH), bf16),
            pltpu.VMEM((NL * TW + 1, 8, DH), bf16),
            kv_buf, kv_buf, kv_buf, kv_buf,
            pltpu.VMEM((8, SK), bf16),
            pltpu.VMEM((H, 8, DH), bf16),
            pltpu.VMEM((DH, DH), f32),
        ],
        compiler_params=pltpu.CompilerParams(
            vmem_limit_bytes=48 * 1024 * 1024, disable_bounds_checks=True),
    )(A_x, kv_t(A_k_cache), kv_t(A_v_cache), A_wq, wo_t(A_wo),
      B_x, kv_t(B_k_cache), kv_t(B_v_cache), B_wq, wo_t(B_wo))
```
